```python
import jax
import jax.numpy as jnp

def _softmax(x, axis=-1):
    return jax.nn.softmax(x, axis=axis)
def _gelu(x):
    return jax.nn.gelu(x, approximate=True)
def _silu(x):
    return jax.nn.silu(x)
def _sigmoid(x):
    return jax.nn.sigmoid(x)
def _layernorm(x, axis=-1, eps=1e-5):
    m = jnp.mean(x, axis=axis, keepdims=True)
    v = jnp.var(x, axis=axis, keepdims=True)
    return (x - m) / jnp.sqrt(v + eps)
def _scatter_add(tgt, idx, src, axis=0):
    return tgt.at[idx].add(src)
def _segment_sum(src, seg, n):
    return jax.ops.segment_sum(src, seg, n)
class _Rng:
    def __init__(self, key):
        self._k = key
    def _next(self):
        self._k, sub = jax.random.split(self._k)
        return sub
    def normal(self, shape):
        return jax.random.normal(self._next(), shape, dtype=jnp.bfloat16)
    def randint(self, lo, hi, shape):
        return jax.random.randint(self._next(), shape, lo, hi, dtype=jnp.int32)
    def uniform(self, shape, lo=0.0, hi=1.0):
        return jax.random.uniform(self._next(), shape, jnp.bfloat16, lo, hi)
    def permutation(self, n):
        return jax.random.permutation(self._next(), n)


kernel_name = 'gated_mix__sliding_block_cached__glu_gated_swiglu__decode'

def setup_inputs():
    _rng = _Rng(jax.random.key(int.from_bytes(__import__("os").urandom(4), "little")))
    _w = (lambda a: (lambda t: t.astype(jnp.bfloat16) if jnp.issubdtype(t.dtype, jnp.floating) else t)(jnp.asarray(a)))
    def _A_setup():
        B, Sq, D = 1, 1, 640
        Hq, Hkv, Sk, Dh = 32, 32, 32768, 192
        assert Hq % Hkv == 0, (Hq, Hkv)
        return {
            "x": _w((lambda *s: _rng.normal(s) * 0.05)(B, Sq, D)),
            "k_cache": _w((lambda *s: _rng.normal(s) * 0.05)(B, Hkv, Sk, Dh)),
            "v_cache": _w((lambda *s: _rng.normal(s) * 0.05)(B, Hkv, Sk, Dh)),
            "wq": _w((lambda *s: _rng.normal(s) * 0.05)(D, Hq * Dh) * (D ** -0.5)),
            "wo": _w((lambda *s: _rng.normal(s) * 0.05)(Hq * Dh, D) * ((Hq * Dh) ** -0.5)),
        }
    _A_in = _A_setup()

    def _B_setup():
        B, S, D, F = 1, 1, 640, 1536
        return {
            "x": _w((lambda *s: _rng.normal(s) * 0.05)(B, S, D)),
            "w1": _w((lambda *s: _rng.normal(s) * 0.05)(D, F) * (2.0 / D) ** 0.5),
            "w3": _w((lambda *s: _rng.normal(s) * 0.05)(D, F) * (2.0 / D) ** 0.5),
            "w2": _w((lambda *s: _rng.normal(s) * 0.05)(F, D) * (2.0 / F) ** 0.5),
        }
    _B_in = _B_setup()

    return {
        "A_x": _A_in["x"],
        "A_k_cache": _A_in["k_cache"],
        "A_v_cache": _A_in["v_cache"],
        "A_wq": _A_in["wq"],
        "A_wo": _A_in["wo"],
        "B_x": _B_in["x"],
        "B_w1": _B_in["w1"],
        "B_w3": _B_in["w3"],
        "B_w2": _B_in["w2"],
        "gate_w": _w((lambda *s: _rng.normal(s) * 0.05)(640)),
    }

def reference(A_x, A_k_cache, A_v_cache, A_wq, A_wo, B_x, B_w1, B_w3, B_w2, gate_w):
    def _A_ref(x, k_cache, v_cache, wq, wo):
        B, Sq, D = x.shape
        Hq, Dh = 32, 192
        Hkv, Sk = k_cache.shape[1], k_cache.shape[2]
        W = min(4096, max(256, Sk // 4))
        rep = Hq // Hkv
        q = (lambda x, *d: x.transpose(*d))((x @ wq).reshape(B, Sq, Hq, Dh), 0, 2, 1, 3)
        k = jnp.repeat(k_cache[:, :, Sk - W:, :], rep, axis=1)
        v = jnp.repeat(v_cache[:, :, Sk - W:, :], rep, axis=1)
        scores = jnp.einsum("bhqd,bhkd->bhqk", q, k) * (Dh ** -0.5)
        p = _softmax(scores, axis=-1)
        o = jnp.einsum("bhqk,bhkd->bhqd", p, v)
        return (lambda x, *d: x.transpose(*d))(o, 0, 2, 1, 3).reshape(B, Sq, Hq * Dh) @ wo

    def _B_ref(x, w1, w3, w2):
        gate = jnp.einsum("bsd,df->bsf", x, w1)
        up = jnp.einsum("bsd,df->bsf", x, w3)
        h = _silu(gate) * up
        out = jnp.einsum("bsf,fd->bsd", h, w2)
        return out

    x = A_x
    g = _sigmoid((x * gate_w).sum(-1, keepdims=True))
    a = _A_ref(x, A_k_cache, A_v_cache, A_wq, A_wo)
    b = _B_ref(x, B_w1, B_w3, B_w2)
    return g * a + (1 - g) * b
```

```python
import jax
import jax.numpy as jnp
from jax import lax
import jax.experimental.pallas as pl
import jax.experimental.pallas.tpu as pltpu

_HQ = 32
_DH = 192


@jax.jit
def pallas_gated_mix__sliding_block_cached__glu_gated_swiglu__decode_kernel(
    A_x: jax.Array,
    A_k_cache: jax.Array,
    A_v_cache: jax.Array,
    A_wq: jax.Array,
    A_wo: jax.Array,
    B_x: jax.Array,
    B_w1: jax.Array,
    B_w3: jax.Array,
    B_w2: jax.Array,
    gate_w: jax.Array,
):
    del B_x
    f32, bf16 = jnp.float32, jnp.bfloat16
    D = A_x.shape[-1]
    H, SK, DH = A_k_cache.shape[1], A_k_cache.shape[2], A_k_cache.shape[3]
    F = B_w1.shape[1]
    assert (H, DH) == (_HQ, _DH)
    W = min(4096, max(256, SK // 4))
    HP = H // 2
    P2 = 2 * DH
    depth = 3

    def kernel(x_hbm, k_hbm, v_hbm, wq_hbm, wo_hbm, w1_hbm, w3_hbm, w2_hbm, gw_hbm, o_ref,
               xb, gwb, wqb, wob, w1b, w3b, w2b, kb, vb, ob, ssem, wsem, ksem, vsem, osem):
        def kcopy(hp, slot):
            return pltpu.make_async_copy(k_hbm.at[0, pl.ds(2 * hp, 2), :, pl.ds(SK - W, W)], kb.at[slot], ksem.at[slot])

        def vcopy(hp, slot):
            return pltpu.make_async_copy(v_hbm.at[0, pl.ds(2 * hp, 2), :, pl.ds(SK - W, W)], vb.at[slot], vsem.at[slot])

        def wocopy(hp):
            return pltpu.make_async_copy(wo_hbm.at[pl.ds(pl.multiple_of(hp * P2, P2), P2), :], wob.at[hp], osem.at[hp])

        c_x = pltpu.make_async_copy(x_hbm, xb, ssem.at[0])
        c_gw = pltpu.make_async_copy(gw_hbm, gwb, ssem.at[1])
        c_wq = pltpu.make_async_copy(wq_hbm, wqb, wsem.at[0])
        c_w1 = pltpu.make_async_copy(w1_hbm, w1b, wsem.at[1])
        c_w3 = pltpu.make_async_copy(w3_hbm, w3b, wsem.at[2])
        c_w2 = pltpu.make_async_copy(w2_hbm, w2b, wsem.at[3])
        c_x.start(); c_gw.start(); c_w1.start(); c_w3.start(); c_w2.start(); c_wq.start()
        for s in range(depth):
            kcopy(s, s).start(); vcopy(s, s).start()

        c_x.wait(); c_gw.wait()
        x1 = xb[0]
        x8 = jnp.broadcast_to(x1, (16, D))
        gw = gwb[...].astype(f32).reshape(1, D)
        g = jax.nn.sigmoid(jnp.sum(x1.astype(f32) * gw, axis=-1, keepdims=True))
        c_w1.wait()
        gate = jnp.dot(x8, w1b[...], preferred_element_type=f32)
        c_w3.wait()
        up = jnp.dot(x8, w3b[...], preferred_element_type=f32)
        hmid = (gate * jax.nn.sigmoid(gate) * up).astype(bf16)
        c_w2.wait()
        bout = jnp.dot(hmid, w2b[...], preferred_element_type=f32)[0:1]
        c_wq.wait()

        row = lax.broadcasted_iota(jnp.int32, (16, P2), 0)
        col = lax.broadcasted_iota(jnp.int32, (16, P2), 1)
        mask = ((row % 2) == 0) == (col < DH)
        scale = DH ** -0.5

        def body(hp, carry):
            slot = hp % depth
            q2 = jnp.dot(x8, wqb[:, pl.ds(pl.multiple_of(hp * P2, P2), P2)], preferred_element_type=f32)
            q2 = jnp.where(mask, q2, 0.0).astype(bf16)
            kcopy(hp, slot).wait()
            k2 = kb[slot].reshape(P2, W)
            s = jnp.dot(q2, k2, preferred_element_type=f32) * scale
            m = jnp.max(s, axis=-1, keepdims=True)
            e = jnp.exp(s - m)
            l = jnp.sum(e, axis=-1, keepdims=True)
            vcopy(hp, slot).wait()
            v2 = vb[slot].reshape(P2, W)
            o2 = lax.dot_general(e.astype(bf16), v2, (((1,), (1,)), ((), ())), preferred_element_type=f32)
            o2 = jnp.where(mask, o2 / l, 0.0)
            ob[hp] = o2.astype(bf16)

            @pl.when(hp + depth < HP)
            def _():
                kcopy(hp + depth, slot).start()
                vcopy(hp + depth, slot).start()

            @pl.when(hp + depth == HP)
            def _():
                for j in range(HP):
                    wocopy(j).start()

            return carry

        lax.fori_loop(0, HP, body, 0)

        def body2(hp, acc):
            wocopy(hp).wait()
            return acc + jnp.dot(ob[hp], wob[hp], preferred_element_type=f32)

        acc = lax.fori_loop(0, HP, body2, jnp.zeros((16, D), f32))
        a = acc[0:1] + acc[1:2]
        o_ref[0] = (g * a + (1.0 - g) * bout).astype(o_ref.dtype)

    kT = jnp.swapaxes(A_k_cache, 2, 3)
    vT = jnp.swapaxes(A_v_cache, 2, 3)
    anyspec = pl.BlockSpec(memory_space=pl.ANY)
    return pl.pallas_call(
        kernel,
        in_specs=[anyspec] * 9,
        out_specs=pl.BlockSpec(memory_space=pltpu.VMEM),
        out_shape=jax.ShapeDtypeStruct((1, 1, D), bf16),
        scratch_shapes=[
            pltpu.VMEM((1, 1, D), bf16), pltpu.VMEM((D,), bf16),
            pltpu.VMEM((D, H * DH), bf16), pltpu.VMEM((HP, P2, D), bf16),
            pltpu.VMEM((D, F), bf16), pltpu.VMEM((D, F), bf16), pltpu.VMEM((F, D), bf16),
            pltpu.VMEM((depth, 2, DH, W), bf16), pltpu.VMEM((depth, 2, DH, W), bf16),
            pltpu.VMEM((HP, 16, P2), bf16),
            pltpu.SemaphoreType.DMA((2,)), pltpu.SemaphoreType.DMA((4,)),
            pltpu.SemaphoreType.DMA((depth,)), pltpu.SemaphoreType.DMA((depth,)), pltpu.SemaphoreType.DMA((HP,)),
        ],
        compiler_params=pltpu.CompilerParams(vmem_limit_bytes=100 * 1024 * 1024),
    )(A_x, kT, vT, A_wq, A_wo, B_w1, B_w3, B_w2, gate_w)
```

```python
import jax
import jax.numpy as jnp
from jax import lax
import jax.experimental.pallas as pl
import jax.experimental.pallas.tpu as pltpu

_M = 16
_NJ = 8
_PIECE_COLS = 2048
_PIECE_TILES = 16
_WO_GROUPS = ((0, 16), (16, 32), (32, 40), (40, 45), (45, 48))


def _tile_view(w):
    r, c = w.shape
    return w.reshape(r // 8, 8, c // 128, 128).transpose(0, 2, 1, 3).reshape(r * c // 1024, 8, 128)


@jax.jit
def pallas_gated_mix__sliding_block_cached__glu_gated_swiglu__decode_kernel(
    A_x: jax.Array,
    A_k_cache: jax.Array,
    A_v_cache: jax.Array,
    A_wq: jax.Array,
    A_wo: jax.Array,
    B_x: jax.Array,
    B_w1: jax.Array,
    B_w3: jax.Array,
    B_w2: jax.Array,
    gate_w: jax.Array,
):
    del B_x
    f32, bf16 = jnp.float32, jnp.bfloat16
    D = A_x.shape[-1]
    _, H, SK, DH = A_k_cache.shape
    F = B_w1.shape[1]
    W = min(4096, max(256, SK // 4))
    assert A_x.shape == (1, 1, 640) and (H, DH, W, F) == (32, 192, 4096, 1536)
    assert A_wq.shape == (D, H * DH) and A_wo.shape == (H * DH, D)
    HP = H // 2
    P2 = 2 * DH
    M, NJ, PC, TP = _M, _NJ, _PIECE_COLS, _PIECE_TILES
    CK = W // NJ
    DT, FT, QT = D // 128, F // 128, H * DH // 128
    groups = _WO_GROUPS
    scale = DH ** -0.5

    def body(x_hbm, k_hbm, v_hbm, wq_hbm, wo_hbm, w1_hbm, w3_hbm, w2_hbm, gw_hbm, o_ref,
             xb, gwb, wqb, wob, w1b, w3b, w2b, kb, vb, qb, sb, ob,
             ssem, wsem, ksem, vsem, osem):

        def loop(n, fn):
            def step(j, carry):
                fn(j)
                return carry
            lax.fori_loop(0, n, step, 0)

        def wait_all(buf, sem):
            pltpu.make_async_copy(buf, buf, sem).wait()

        def piece(src, dst, sem, k, prio, tp=TP):
            rows = pl.ds(pl.multiple_of(k * tp, tp), tp)
            pltpu.async_copy(src.at[rows], dst.at[rows], sem, priority=prio)

        def kv_step(src, buf, sem, p, j):
            slot = p % 2
            c, h = j // 4, (j % 4) // 2
            for i in range(12):
                r = 12 * (j % 2) + i
                pltpu.async_copy(
                    src.at[0, 2 * p + h, pl.ds(pl.multiple_of(8 * r, 8), 8),
                           pl.ds(pl.multiple_of(SK - W + c * PC, PC), PC)],
                    buf.at[slot, pl.ds(pl.multiple_of(DH * h + 8 * r, 8), 8),
                           pl.ds(pl.multiple_of(c * PC, PC), PC)],
                    sem.at[slot], priority=i % 2)

        def wq_step(o):
            for half in range(2):
                for i in range(15):
                    piece(wq_hbm, wqb, wsem.at[0], 2 * o + half + 16 * i, (15 * half + i) % 2)

        def wo_step(t):
            @pl.when(t < 15)
            def _():
                for i in range(16):
                    q = 16 * t + i
                    ql = q - jnp.where(q < 80, 0, 80)
                    k = jnp.where(q < 160, (q - ql) + ql // 5 + 16 * (ql % 5), q)
                    g = 0
                    for k0, _ in groups[1:]:
                        g = g + jnp.where(k >= DT * k0, 1, 0)
                    piece(wo_hbm, wob, osem.at[g], k, i % 2)

        def cat_tiles(ref, base, stride, n):
            return jnp.concatenate([ref[base + stride * i] for i in range(n)], axis=0)

        pltpu.async_copy(x_hbm, xb, ssem.at[0])
        pltpu.async_copy(gw_hbm, gwb, ssem.at[1])

        def mlp_issue(o):
            for i in range(4):
                for a, (src, dst) in enumerate(((w1_hbm, w1b), (w3_hbm, w3b), (w2_hbm, w2b))):
                    piece(src, dst, wsem.at[1 + a], o + 30 * i, (3 * i + a) % 2, TP // 2)
        loop(30, mlp_issue)
        loop(3, wq_step)

        wait_all(xb, ssem.at[0])
        wait_all(gwb, ssem.at[1])
        x1 = xb[0]
        xm = jnp.broadcast_to(x1, (M, D))
        gw = gwb[...].astype(f32).reshape(1, D)
        gate_g = jax.nn.sigmoid(jnp.sum(x1.astype(f32) * gw, axis=-1, keepdims=True))
        wait_all(w1b, wsem.at[1])
        wait_all(w3b, wsem.at[2])
        wait_all(w2b, wsem.at[3])

        def mlp_step(j, bacc):
            gate = jnp.dot(xm, cat_tiles(w1b, j, FT, D // 8), preferred_element_type=f32)
            up = jnp.dot(xm, cat_tiles(w3b, j, FT, D // 8), preferred_element_type=f32)
            hid = (gate * jax.nn.sigmoid(gate) * up).astype(bf16)
            w2j = jnp.concatenate([cat_tiles(w2b, 16 * DT * j + ct, DT, 16) for ct in range(DT)], axis=1)
            bacc = bacc + jnp.dot(hid, w2j, preferred_element_type=f32)

            @pl.when(j < 5)
            def _():
                wq_step(3 + j)
            return bacc
        b_out = lax.fori_loop(0, FT, mlp_step, jnp.zeros((M, D), f32))[0:1]

        loop(NJ, lambda j: kv_step(k_hbm, kb, ksem, 0, j))
        wait_all(wqb, wsem.at[0])
        row = lax.broadcasted_iota(jnp.int32, (M, P2), 0)
        col = lax.broadcasted_iota(jnp.int32, (M, P2), 1)
        own = ((row % 2) == 0) == (col < DH)

        def q_step(p):
            wqp = jnp.concatenate([cat_tiles(wqb, 3 * p + u, QT, D // 8) for u in range(3)], axis=1)
            q2 = jnp.dot(xm, wqp, preferred_element_type=f32)
            qb[:, pl.ds(pl.multiple_of(p * P2, P2), P2)] = jnp.where(own, q2, 0.0).astype(bf16)

            @pl.when(p % 2 == 0)
            def _():
                kv_step(v_hbm, vb, vsem, 0, p // 2)
        loop(HP, q_step)

        def feed(src, buf, sem, p, j, phase):
            @pl.when(p + 1 < HP)
            def _():
                kv_step(src, buf, sem, p + 1, j)

            @pl.when(p + 1 == HP)
            def _():
                wo_step(phase * NJ + j)

        def pair_step(p):
            slot = p % 2
            c0 = pl.multiple_of(p * P2, P2)
            q2 = qb[:, pl.ds(c0, P2)]
            wait_all(kb.at[slot], ksem.at[slot])

            def k_step(j, mrun):
                k0 = pl.multiple_of(j * CK, CK)
                s = jnp.dot(q2, kb[slot, :, pl.ds(k0, CK)], preferred_element_type=f32) * scale
                sb[:, pl.ds(k0, CK)] = s
                for t in range(CK // 128):
                    mrun = jnp.maximum(mrun, s[:, t * 128:(t + 1) * 128])
                feed(k_hbm, kb, ksem, p, j, 0)
                return mrun
            mrun = lax.fori_loop(0, NJ, k_step, jnp.full((M, 128), -jnp.inf, f32))
            m = jnp.max(mrun, axis=-1, keepdims=True)
            wait_all(vb.at[slot], vsem.at[slot])

            def v_step(j, carry):
                lrun, oacc = carry
                k0 = pl.multiple_of(j * CK, CK)
                e = jnp.exp(sb[:, pl.ds(k0, CK)] - m)
                for t in range(CK // 128):
                    lrun = lrun + e[:, t * 128:(t + 1) * 128]
                oacc = oacc + lax.dot_general(
                    e.astype(bf16), vb[slot, :, pl.ds(k0, CK)], (((1,), (1,)), ((), ())),
                    preferred_element_type=f32)
                feed(v_hbm, vb, vsem, p, j, 1)
                return lrun, oacc
            lrun, oacc = lax.fori_loop(
                0, NJ, v_step, (jnp.zeros((M, 128), f32), jnp.zeros((M, P2), f32)))
            l = jnp.sum(lrun, axis=-1, keepdims=True)
            ob[:, pl.ds(c0, P2)] = jnp.where(own, oacc / l, 0.0).astype(bf16)
        loop(HP, pair_step)

        def wo_rows(kt, n):
            return jnp.concatenate(
                [cat_tiles(wob, 16 * DT * kt + ct, DT, 16 * n) for ct in range(DT)], axis=1)

        acc = jnp.zeros((M, D), f32)
        for gi, (k0, k1) in enumerate(groups):
            wait_all(wob.at[pl.ds(16 * DT * k0, 16 * DT * (k1 - k0))], osem.at[gi])
            if k1 - k0 > 8:
                def o_step(kt, acc):
                    lhs = ob[:, pl.ds(pl.multiple_of(kt * 256, 256), 256)]
                    return acc + jnp.dot(lhs, wo_rows(2 * kt, 2), preferred_element_type=f32)
                acc = lax.fori_loop(k0 // 2, k1 // 2, o_step, acc)
            else:
                acc = acc + jnp.dot(ob[:, 128 * k0:128 * k1], wo_rows(k0, k1 - k0),
                                    preferred_element_type=f32)
        a_out = acc[0:1] + acc[1:2]
        o_ref[0] = (gate_g * a_out + (1.0 - gate_g) * b_out).astype(o_ref.dtype)

    kT = jnp.swapaxes(A_k_cache, 2, 3)
    vT = jnp.swapaxes(A_v_cache, 2, 3)
    ws = [_tile_view(w) for w in (A_wq, A_wo, B_w1, B_w3, B_w2)]
    hbm = pl.BlockSpec(memory_space=pl.ANY)
    dma = pltpu.SemaphoreType.DMA
    return pl.pallas_call(
        body,
        in_specs=[hbm] * 9,
        out_specs=pl.BlockSpec(memory_space=pltpu.VMEM),
        out_shape=jax.ShapeDtypeStruct(A_x.shape, A_x.dtype),
        scratch_shapes=[
            pltpu.VMEM((1, 1, D), bf16), pltpu.VMEM((D,), bf16),
            *[pltpu.VMEM(w.shape, bf16) for w in ws],
            pltpu.VMEM((2, P2, W), bf16), pltpu.VMEM((2, P2, W), bf16),
            pltpu.VMEM((M, H * DH), bf16),
            pltpu.VMEM((M, W), f32),
            pltpu.VMEM((M, H * DH), bf16),
            dma((2,)), dma((4,)), dma((2,)), dma((2,)), dma((len(groups),)),
        ],
        compiler_params=pltpu.CompilerParams(
            vmem_limit_bytes=64 * 1024 * 1024,
            disable_bounds_checks=True,
            disable_semaphore_checks=True,
        ),
    )(A_x, kT, vT, *ws, gate_w)
```
